```python
import os as _os
_os.environ.setdefault("JAX_PLATFORMS", "cpu")
import jax
import jax.numpy as jnp

def _softmax(x, axis=-1):
    return jax.nn.softmax(x, axis=axis)
def _gelu(x):
    return jax.nn.gelu(x, approximate=True)
def _silu(x):
    return jax.nn.silu(x)
def _sigmoid(x):
    return jax.nn.sigmoid(x)
def _layernorm(x, axis=-1, eps=1e-5):
    m = jnp.mean(x, axis=axis, keepdims=True)
    v = jnp.var(x, axis=axis, keepdims=True)
    return (x - m) / jnp.sqrt(v + eps)
def _scatter_add(tgt, idx, src, axis=0):
    return tgt.at[idx].add(src)
def _segment_sum(src, seg, n):
    return jax.ops.segment_sum(src, seg, n)
class _Rng:
    def __init__(self, key):
        self._k = key
    def _next(self):
        self._k, sub = jax.random.split(self._k)
        return sub
    def normal(self, shape):
        return jax.random.normal(self._next(), shape, dtype=jnp.bfloat16)
    def randint(self, lo, hi, shape):
        return jax.random.randint(self._next(), shape, lo, hi, dtype=jnp.int32)
    def uniform(self, shape, lo=0.0, hi=1.0):
        return jax.random.uniform(self._next(), shape, jnp.bfloat16, lo, hi)
    def permutation(self, n):
        return jax.random.permutation(self._next(), n)


kernel_name = 'concat_heads__linear_attn_block__sliding_local_dilated__prompt'

def setup_inputs():
    _rng = _Rng(jax.random.key(int.from_bytes(__import__("os").urandom(4), "little")))
    _w = (lambda a: (lambda t: t.astype(jnp.bfloat16) if jnp.issubdtype(t.dtype, jnp.floating) else t)(jnp.asarray(a)))
    def _A_setup():
        B, S, D = 1, 2048, 576
        return {
            "x": _w((lambda *s: _rng.normal(s) * 0.05)(B, S, D)),
            "wqkv": _w((lambda *s: _rng.normal(s) * 1.6)(D, 3 * D)),
            "wo": _w((lambda *s: _rng.normal(s) * 0.4)(D, D)),
        }
    _A_in = _A_setup()

    def _B_setup():
        B, S, D = 1, 2048, 576
        return {
            "x": _w((lambda *s: _rng.normal(s) * 0.2)(B, S, D)),
            "wqkv": _w((lambda *s: _rng.normal(s) * 0.2)(D, 3 * D)),
            "wo": _w((lambda *s: _rng.normal(s) * 0.05)(D, D)),
        }
    _B_in = _B_setup()

    return {
        "A_x": _A_in["x"],
        "A_wqkv": _A_in["wqkv"],
        "A_wo": _A_in["wo"],
        "B_x": _B_in["x"],
        "B_wqkv": _B_in["wqkv"],
        "B_wo": _B_in["wo"],
    }

def reference(A_x, A_wqkv, A_wo, B_x, B_wqkv, B_wo):
    def _A_ref(x, wqkv, wo):
        B, S, D = x.shape
        H = 32; Dh = D // H
        qkv = (lambda x, *d: x.transpose(*d))((x @ wqkv).reshape(B, S, 3, H, Dh), 2, 0, 3, 1, 4)
        q, k, v = qkv[0], qkv[1], qkv[2]
        phi = lambda t: jnp.where(t > 0, t + 1, jnp.exp(t)) + 1e-6
        pq, pk = phi(q), phi(k)
        kv = jnp.einsum("bhsd,bhse->bhde", pk, v)
        z = jnp.einsum("bhsd->bhd", pk)
        num = jnp.einsum("bhqd,bhde->bhqe", pq, kv)
        den = jnp.einsum("bhqd,bhd->bhq", pq, z)[..., None] + 1e-6
        o = num / den
        return (lambda x, *d: x.transpose(*d))(o, 0, 2, 1, 3).reshape(B, S, D) @ wo

    def _B_ref(x, wqkv, wo):
        B, S, D = x.shape
        H = 32; Dh = D // H
        W, dil = 8, 2
        qkv = (lambda x, *d: x.transpose(*d))((x @ wqkv).reshape(B, S, 3, H, Dh), 2, 0, 3, 1, 4)
        q, k, v = qkv[0], qkv[1], qkv[2]
        scale = Dh ** -0.5
        pos = jnp.arange(S)
        off = jnp.arange(W) * dil
        idx = pos[:, None] - off[None, :]
        mask = idx >= 0
        idx_c = jnp.where(mask, idx, 0).reshape(-1)
        kg = k[:, :, idx_c, :].reshape(B, H, S, W, Dh)
        vg = v[:, :, idx_c, :].reshape(B, H, S, W, Dh)
        logits = jnp.einsum("bhsd,bhswd->bhsw", q, kg) * scale
        logits = jnp.where(mask[None, None, :, :], logits, -1e9)
        attn = _softmax(logits, axis=-1)
        o = jnp.einsum("bhsw,bhswd->bhsd", attn, vg)
        return (lambda x, *d: x.transpose(*d))(o, 0, 2, 1, 3).reshape(B, S, D) @ wo

    a = _A_ref(A_x, A_wqkv, A_wo)
    b = _B_ref(B_x, B_wqkv, B_wo)
    return jnp.concatenate([a, b], axis=-1)
```

```python
import os
import jax
import jax.numpy as jnp
from jax.experimental import pallas as pl
from jax.experimental.pallas import tpu as pltpu

S, D, H, DH = int(os.environ.get("KS", 2048)), 576, 32, 18
DP = 640
NW, DIL = 8, 2
HALO = 16
BF, F32, U32 = jnp.bfloat16, jnp.float32, jnp.uint32
NT = (((1,), (1,)), ((), ()))
LOG2E = 1.4426950408889634

RB = 256
NB = S // RB
R1 = 512
N1 = S // R1
GR = 16
FC = 64
NFC = RB // FC


def _phi(t):
    return jnp.where(t > 0, t + 1.0, jnp.exp(t)) + 1e-6


def _kernel(xa_h, wa_h, woa_h, xb_h, wb_h, wob_h, o_h,
            xa, xb, wa, wb, woa, wob, ta, tb, t2, waT, wbT, woT, wobP,
            g_acc, kvm, mT, zb, kb0, kb1, vb0, vb1, qb0, qb1, obuf, xn0, xn1, pk0, pk1, pbuf, outs, fold,
            sem_in, sem_out):
    kbufs, vbufs, qbufs, xns, pks = (kb0, kb1), (vb0, vb1), (qb0, qb1), (xn0, xn1), (pk0, pk1)
    ins = []

    def cp(src, dst):
        c = pltpu.make_async_copy(src, dst, sem_in.at[len(ins)])
        ins.append(c)
        return c

    c_wak = cp(wa_h.at[:, pl.ds(512, 640)], wa.at[pl.ds(0, D), pl.ds(512, 640)])
    c_xa = [cp(xa_h.at[:, pl.ds(i * R1, R1)], xa.at[pl.ds(0, D), pl.ds(i * R1, R1)]) for i in range(N1)]
    c_waq = cp(wa_h.at[:, pl.ds(0, 512)], wa.at[pl.ds(0, D), pl.ds(0, 512)])
    c_wb = cp(wb_h, wb.at[pl.ds(0, D), :])
    c_wav = cp(wa_h.at[:, pl.ds(1152, 576)], wa.at[pl.ds(0, D), pl.ds(1152, 576)])
    c_woa = cp(woa_h, woa)
    c_wob = cp(wob_h, wob)
    c_xb = [cp(xb_h.at[:, pl.ds(i * R1, R1)], xb.at[pl.ds(0, D), pl.ds(i * R1, R1)]) for i in range(N1)]
    out_copies = [pltpu.make_async_copy(outs.at[pl.ds(i * RB, RB), :], o_h.at[pl.ds(i * RB, RB), :], sem_out.at[i])
                  for i in range(NB)]

    c_wak.start()
    c_xa[0].start()

    wa[pl.ds(D, DP - D), :] = jnp.zeros((DP - D, 3 * D), BF)
    xa[pl.ds(D, DP - D), :] = jnp.ones((DP - D, S), BF)

    def init_late():
        xb[pl.ds(D, DP - D), :] = jnp.zeros((DP - D, S), BF)
        wb[pl.ds(D, DP - D), :] = jnp.zeros((DP - D, 3 * D), BF)
        for j in range(5):
            kb0[j, pl.ds(0, HALO), :] = jnp.zeros((HALO, 128), F32)
            vb0[j, pl.ds(0, HALO), :] = jnp.zeros((HALO, 128), F32)
        kvm[...] = jnp.zeros((D, DP), BF)
        li = jax.lax.broadcasted_iota(jnp.int32, (128, 128), 0)
        lj = jax.lax.broadcasted_iota(jnp.int32, (128, 128), 1)
        fold[...] = jnp.where(((li & 63) >> 1) == ((lj & 63) >> 1), 1.0, 0.0).astype(BF)
        wbT[pl.ds(1728, 64), :] = jnp.zeros((64, DP), BF)
        wobP[pl.ds(512, 64), :] = jnp.zeros((64, DP), BF)

    def xpose_w(w_ref, t_ref, c0, c1, kt):
        blk = w_ref[pl.ds(128 * kt, 128), pl.ds(c0, c1 - c0)]
        t_ref[kt, pl.ds(c0 // 2, (c1 - c0) // 2), :] = pltpu.bitcast(blk.T, U32)

    def gather_rows(t_ref, dst, src0, nh, dst0, kt):
        v = t_ref[kt, pl.ds(src0, nh, stride=9), :]
        dst.bitcast(U32)[pl.ds(dst0 // 2, nh), pl.ds(128 * kt, 128)] = v

    def prep_a(part, kt):
        for g in range(4):
            for c in range(9):
                gather_rows(ta, waT, part * 288 + 72 * g + c, 8, part * D + 144 * g + 16 * c, kt)

    def prep_b_x(kt):
        xpose_w(wb, tb, 0, 3 * D, kt)

    def prep_b_g(kt):
        for part in range(3):
            for c in range(8):
                gather_rows(tb, wbT, part * 288 + c, 32, part * 512 + 64 * c, kt)
        gather_rows(tb, wbT, 0 * 288 + 8, 32, 1536, kt)
        gather_rows(tb, wbT, 2 * 288 + 8, 32, 1600, kt)
        gather_rows(tb, wbT, 1 * 288 + 8, 32, 1664, kt)

    def prep_wob():
        for jt in range(5):
            w = min(128, D - 128 * jt)
            t2[jt, :, pl.ds(0, w)] = pltpu.bitcast(wob[:, pl.ds(128 * jt, w)], U32)
        lane = jax.lax.broadcasted_iota(jnp.int32, (32, 128), 1)
        for c in range(9):
            prev = None
            dst0 = 64 * c if c < 8 else 576
            for jt in range(5):
                v = t2[jt, pl.ds(c, 32, stride=9), :]
                if jt == 4:
                    v = jnp.where(lane < 64, v, jnp.uint32(0))
                r = pltpu.roll(v, 64, 1)
                lo = jnp.zeros_like(r) if prev is None else prev
                wobP.bitcast(U32)[pl.ds(dst0 // 2, 32), pl.ds(128 * jt, 128)] = jnp.where(lane < 64, lo, r)
                prev = r

    def a_k(i, g):
        xs = xa[:, pl.ds(i * R1, R1)]
        kT = jnp.dot(waT[pl.ds(D + 144 * g, 144), :], xs, preferred_element_type=F32)
        pks[i % 2][pl.ds(144 * g, 144), :] = _phi(kT).astype(BF)

    def a_g(i, j):
        xs = xa[pl.ds(128 * j, 128), pl.ds(i * R1, R1)]
        gp = jax.lax.dot_general(pks[i % 2][...], xs, NT, preferred_element_type=F32)
        if i == 0:
            g_acc[:, pl.ds(128 * j, 128)] = gp
        else:
            g_acc[:, pl.ds(128 * j, 128)] += gp

    groups = [(0,), (0, 1), (1, 2), (2, 3), (3,)]
    krange = [(0, 256), (0, 384), (128, 512), (256, 576), (384, 576)]

    def a_z():
        zb[...] = jnp.broadcast_to(g_acc[:, pl.ds(D, 1)], (D, 128))

    def a_kv(j):
        w = min(128, D - 128 * j)
        wv = wa[:, pl.ds(2 * D + 128 * j, w)]
        for g in groups[j]:
            gb = g_acc[pl.ds(144 * g, 144), :].astype(BF)
            kv = jnp.dot(gb, wv, preferred_element_type=F32)
            r = jax.lax.broadcasted_iota(jnp.int32, (144, w), 0)
            n = jax.lax.broadcasted_iota(jnp.int32, (144, w), 1) + 128 * j
            lo = ((r & 15) >> 1) * DH + 144 * g
            kvm[pl.ds(144 * g, 144), pl.ds(128 * j, w)] = jnp.where((n >= lo) & (n < lo + DH), kv, 0.0).astype(BF)

    def a_m(j):
        w = min(128, D - 128 * j)
        k0, k1 = krange[j]
        m = jax.lax.dot_general(woT[:, pl.ds(k0, k1 - k0)], kvm[pl.ds(128 * j, w), pl.ds(k0, k1 - k0)], NT,
                                preferred_element_type=F32)
        mT[:, pl.ds(128 * j, w)] = m.astype(BF)

    cscale = (DH ** -0.5) * LOG2E

    def b_xn(i):
        xns[i % 2][...] = xb[:, pl.ds(i * RB, RB)].T

    def b_proj(i, p):
        kbuf, vbuf, qbuf = kbufs[i % 2], vbufs[i % 2], qbufs[i % 2]
        rows = pl.ds(HALO, RB)
        res = jax.lax.dot_general(xns[i % 2][...], wbT[pl.ds(256 * p, 256), :], NT, preferred_element_type=F32)
        for t in range(2):
            v = res[:, 128 * t:128 * t + 128]
            j = 2 * (p % 2) + t
            if p < 2:
                qbuf[j] = v
            elif p < 4:
                kbuf[j, rows, :] = v
            elif p < 6:
                vbuf[j, rows, :] = v
            elif t == 0:
                vbuf[4, rows, :] = v
            else:
                kbuf[4, rows, :] = v

    def b_halo(i):
        kbuf, vbuf = kbufs[i % 2], vbufs[i % 2]
        kp, vp = kbufs[(i - 1) % 2], vbufs[(i - 1) % 2]
        for j in range(5):
            kbuf[j, pl.ds(0, HALO), :] = kp[j, pl.ds(RB, HALO), :]
            vbuf[j, pl.ds(0, HALO), :] = vp[j, pl.ds(RB, HALO), :]

    vals = {}

    def b_qk(i, c):
        kbuf, vbuf, qbuf = kbufs[i % 2], vbufs[i % 2], qbufs[i % 2]
        accs = []
        for r in range(c * FC, (c + 1) * FC, GR):
            q = [qbuf[j, pl.ds(r, GR), :] for j in range(4)] + [vbuf[4, pl.ds(HALO + r, GR), :]]
            for w in range(NW):
                rs = pl.ds(HALO + r - DIL * w, GR)
                a = q[0] * kbuf[0, rs, :]
                for j in range(1, 5):
                    a = a + q[j] * kbuf[j, rs, :]
                accs.append(a)
        vals["acc", i, c] = jnp.concatenate(accs, axis=0).astype(BF)

    def b_fold(i, c):
        vals["L", i, c] = jnp.dot(vals.pop(("acc", i, c)), fold[...], preferred_element_type=F32)

    def b_av(i, c):
        vbuf = vbufs[i % 2]
        L = vals.pop(("L", i, c))
        for gi, r in enumerate(range(c * FC, (c + 1) * FC, GR)):
            ls = [L[(gi * NW + w) * GR:(gi * NW + w + 1) * GR] for w in range(NW)]
            if i == 0 and r == 0:
                row = jax.lax.broadcasted_iota(jnp.int32, (GR, 128), 0)
                ls = [ls[0]] + [jnp.where(row >= DIL * w, ls[w], -1e30) for w in range(1, NW)]
            m01 = jnp.maximum(jnp.maximum(ls[0], ls[1]), jnp.maximum(ls[2], ls[3]))
            m23 = jnp.maximum(jnp.maximum(ls[4], ls[5]), jnp.maximum(ls[6], ls[7]))
            m = jnp.maximum(m01, m23)
            es = [jnp.exp2((l - m) * cscale) for l in ls]
            s = ((es[0] + es[1]) + (es[2] + es[3])) + ((es[4] + es[5]) + (es[6] + es[7]))
            rinv = pl.reciprocal(s, approx=True)
            os_ = []
            for j in range(5):
                o = es[0] * vbuf[j, pl.ds(HALO + r, GR), :]
                for w in range(1, NW):
                    o = o + es[w] * vbuf[j, pl.ds(HALO + r - DIL * w, GR), :]
                os_.append(o * rinv)
            obuf[pl.ds(r, GR), :] = jnp.concatenate(os_, axis=1).astype(BF)

    def b_out(i, p):
        c0, n = ((0, 256), (256, 256), (512, 128))[p]
        ob = jnp.dot(obuf[...], wobP[:, pl.ds(c0, n)], preferred_element_type=F32)
        outs[pl.ds(i * RB, RB), pl.ds(512 + c0, n)] = ob.astype(BF)

    def a_q(i, g):
        xs = xa[:, pl.ds(i * RB, RB)]
        vals["q", i, g] = jnp.dot(waT[pl.ds(144 * g, 144), :], xs, preferred_element_type=F32)

    def a_p(i, g):
        pq = _phi(vals.pop(("q", i, g)))
        par = jax.lax.broadcasted_iota(jnp.int32, (8, 128), 0) & 1
        cols = []
        for lt in range(RB // 128):
            halves = []
            for hf in range(2):
                t = None
                for c in range(9):
                    r = 16 * c + 8 * hf
                    u = pq[r:r + 8, 128 * lt:128 * lt + 128] * zb[pl.ds(144 * g + r, 8), :]
                    t = u if t is None else t + u
                sw = jnp.where(par == 0, pltpu.roll(t, 7, 0), pltpu.roll(t, 1, 0))
                halves.append(pl.reciprocal(t + sw + 1e-6, approx=True))
            cols.append(jnp.concatenate(halves, axis=0))
        rinv = jnp.concatenate(cols, axis=1)
        pT = jnp.concatenate([pq[16 * c:16 * c + 16] * rinv for c in range(9)], axis=0)
        pbuf[pl.ds(144 * g, 144), :] = pT.astype(BF)

    def a_out(i, t):
        c0, n = ((0, 256), (256, 256), (512, 64))[t]
        oT = jnp.dot(mT[pl.ds(c0, n), pl.ds(0, D)], pbuf[...], preferred_element_type=F32).astype(BF)
        vals["o", i, t] = oT

    def a_store(i, t):
        c0, n = ((0, 256), (256, 256), (512, 64))[t]
        outs[pl.ds(i * RB, RB), pl.ds(c0, n)] = vals.pop(("o", i, t)).T

    c_waq.start()
    for c in c_xa[1:]:
        c.start()
    c_wak.wait()
    for kt in range(5):
        xpose_w(wa, ta, 512, 1152, kt)
        prep_a(1, kt)
    c_xa[0].wait()
    for g in range(4):
        a_k(0, g)
    c_wb.start()
    c_wav.start()
    c_woa.start()
    c_wob.start()
    for c in c_xb:
        c.start()

    side = []
    side.append(lambda: c_waq.wait())
    for kt in range(5):
        side.append(lambda kt=kt: (xpose_w(wa, ta, 0, 512, kt), prep_a(0, kt)))
    side.append(init_late)
    side.append(lambda: c_wb.wait())
    for kt in range(5):
        side.append(lambda kt=kt: prep_b_x(kt))
        side.append(lambda kt=kt: prep_b_g(kt))
    side.append(lambda: (c_wob.wait(), prep_wob()))
    side.append(lambda: (c_woa.wait(), woT.__setitem__(Ellipsis, woa[...].T)))
    side.append(lambda: (c_xb[0].wait(), b_xn(0)))
    side.append(lambda: b_xn(1))

    def pop_side(n=1):
        for _ in range(n):
            if side:
                side.pop(0)()

    for i in range(N1):
        nxt = i + 1 < N1
        if nxt:
            c_xa[i + 1].wait()
        for j in range(5):
            if nxt and j < 4:
                a_k(i + 1, j)
            a_g(i, j)
            pop_side(2 if i > 0 else 1)
    while side:
        pop_side()

    c_wav.wait()
    a_z()
    for p in range(7):
        b_proj(0, p)
        if p < 5:
            a_kv(p)
    pending = []
    for i in range(NB):
        nxt = i + 1 < NB
        if i > 0:
            b_halo(i)

        def P(p):
            if nxt:
                b_proj(i + 1, p)

        P(0); b_qk(i, 0)
        for f in pending:
            f()
        pending = []
        P(1); b_qk(i, 1)
        b_fold(i, 0)
        if i == 0:
            for j in range(5):
                a_m(j)
        P(2); b_qk(i, 2)
        b_fold(i, 1); P(3); b_qk(i, 3)
        b_fold(i, 2); a_q(i, 0); a_q(i, 1); b_av(i, 0)
        b_fold(i, 3); a_q(i, 2); a_q(i, 3); b_av(i, 1)
        P(4); b_av(i, 2)
        P(5); b_av(i, 3)
        P(6); a_p(i, 0); a_p(i, 1)
        b_out(i, 0); a_p(i, 2); a_p(i, 3)
        b_out(i, 1); b_out(i, 2)
        if i + 2 < NB:
            if (i + 2) * RB % R1 == 0:
                c_xb[(i + 2) * RB // R1].wait()
            b_xn(i + 2)
        a_out(i, 0); a_out(i, 1); a_store(i, 0); a_out(i, 2)
        pending = [lambda i=i: a_store(i, 1), lambda i=i: a_store(i, 2), lambda i=i: out_copies[i].start()]
    for f in pending:
        f()
    for c in out_copies:
        c.wait()


def build(interpret=False):
    hbm = pl.BlockSpec(memory_space=pltpu.HBM)
    vm = pltpu.VMEM
    scratch = [
        vm((DP, S), BF), vm((DP, S), BF),
        vm((DP, 3 * D), BF), vm((DP, 3 * D), BF),
        vm((D, D), BF), vm((D, D), BF),
        vm((5, 864, 128), U32), vm((5, 864, 128), U32), vm((5, 288, 128), U32),
        vm((2 * D, DP), BF), vm((1792, DP), BF), vm((D, D), BF), vm((DP, DP), BF),
        vm((D, DP), F32), vm((D, DP), BF), vm((D, DP), BF), vm((D, 128), F32),
        vm((5, HALO + RB, 128), F32), vm((5, HALO + RB, 128), F32),
        vm((5, HALO + RB, 128), F32), vm((5, HALO + RB, 128), F32),
        vm((4, RB, 128), F32), vm((4, RB, 128), F32), vm((RB, DP), BF),
        vm((RB, DP), BF), vm((RB, DP), BF),
        vm((D, R1), BF), vm((D, R1), BF), vm((D, RB), BF),
        vm((S, 2 * D), BF), vm((128, 128), BF),
        pltpu.SemaphoreType.DMA((2 * N1 + 8,)), pltpu.SemaphoreType.DMA((NB,)),
    ]
    return pl.pallas_call(
        _kernel,
        out_shape=jax.ShapeDtypeStruct((S, 2 * D), BF),
        in_specs=[hbm] * 6,
        out_specs=hbm,
        scratch_shapes=scratch,
        compiler_params=pltpu.CompilerParams(vmem_limit_bytes=100 << 20),
        interpret=interpret,
    )


@jax.jit
def pallas_concat_heads__linear_attn_block__sliding_local_dilated__prompt_kernel(A_x, A_wqkv, A_wo, B_x, B_wqkv, B_wo):
    out = build()(A_x.reshape(S, D).T, A_wqkv, A_wo, B_x.reshape(S, D).T, B_wqkv, B_wo)
    return out.reshape(1, S, 2 * D)
```

```python
import jax
import jax.numpy as jnp
from jax.experimental import pallas as pl
from jax.experimental.pallas import tpu as pltpu

S, D, H, DH = 2048, 576, 32, 18
DP = 640
NW, DIL = 8, 2
HALO = 16
BF, F32, U32 = jnp.bfloat16, jnp.float32, jnp.uint32
NT = (((1,), (1,)), ((), ()))
LOG2E = 1.4426950408889634

RB = 256
NB = S // RB
R1 = 512
P1 = [(0, 256), (256, 256)] + [(p, 512) for p in range(512, S, 512)]
N1 = len(P1)
GR = 16
PN = 256
BN = 256
FC = 32
FG = 32
AQM = 144
AOM = 256


def split(n, step):
    return [(c, min(step, n - c)) for c in range(0, n, step)]


PP, BP, AQP, AOP = split(1792, PN), split(DP, BN), split(D, AQM), split(D, AOM)


def _phi(t):
    return jnp.where(t > 0, t + 1.0, jnp.exp(t)) + 1e-6


def _kernel(xa_h, wa_h, woa_h, xb_h, wb_h, wob_h, o_h,
            xa, xb, wa, wb, woa, wob, ta, tb, t2, waT, wbT, woT, wobP,
            g_acc, kvm, mT, zb, kb0, kb1, vb0, vb1, qb0, qb1, ob0, ob1, accb, pk0, pk1, pbuf, outs, fold,
            sem_in, sem_out):
    kbufs, vbufs, qbufs, pks = (kb0, kb1), (vb0, vb1), (qb0, qb1), (pk0, pk1)
    obufs = (ob0, ob1)
    vals = {}
    ins = []

    def cp(src, dst):
        c = pltpu.make_async_copy(src, dst, sem_in.at[len(ins)])
        ins.append(c)
        return c

    c_wak = [cp(wa_h.at[pl.ds(128 * kt, min(128, D - 128 * kt)), pl.ds(512, 640)],
                wa.at[pl.ds(128 * kt, min(128, D - 128 * kt)), pl.ds(512, 640)]) for kt in range(5)]
    c_xa0 = cp(xa_h.at[:, pl.ds(0, 256)], xa.at[pl.ds(0, D), pl.ds(0, 256)])
    c_xa1 = cp(xa_h.at[:, pl.ds(256, 256)], xa.at[pl.ds(0, D), pl.ds(256, 256)])
    c_xa2 = cp(xa_h.at[:, pl.ds(512, 512)], xa.at[pl.ds(0, D), pl.ds(512, 512)])
    c_waq = cp(wa_h.at[:, pl.ds(0, 512)], wa.at[pl.ds(0, D), pl.ds(0, 512)])
    c_xa3 = cp(xa_h.at[:, pl.ds(1024, S - 1024)], xa.at[pl.ds(0, D), pl.ds(1024, S - 1024)])
    c_wb = cp(wb_h, wb.at[pl.ds(0, D), :])
    c_wob = cp(wob_h, wob)
    c_woa = cp(woa_h, woa)
    c_wav = cp(wa_h.at[:, pl.ds(1152, 576)], wa.at[pl.ds(0, D), pl.ds(1152, 576)])
    c_xb = cp(xb_h, xb.at[pl.ds(0, D), :])
    outc = []

    def out_copy(i, c0, n):
        c = pltpu.make_async_copy(outs.at[pl.ds(i * RB, RB), pl.ds(c0, n)], o_h.at[pl.ds(i * RB, RB), pl.ds(c0, n)],
                                  sem_out.at[len(outc)])
        outc.append(c)
        c.start()

    for c in ins:
        c.start()

    wa[pl.ds(D, DP - D), :] = jnp.zeros((DP - D, 3 * D), BF)
    xa[pl.ds(D, DP - D), :] = jnp.ones((DP - D, S), BF)

    def init_late():
        xb[pl.ds(D, DP - D), :] = jnp.zeros((DP - D, S), BF)
        wb[pl.ds(D, DP - D), :] = jnp.zeros((DP - D, 3 * D), BF)
        for j in range(5):
            kb0[j, pl.ds(0, HALO), :] = jnp.zeros((HALO, 128), F32)
        kvm[...] = jnp.zeros((D, DP), BF)
        li = jax.lax.broadcasted_iota(jnp.int32, (128, 128), 0)
        lj = jax.lax.broadcasted_iota(jnp.int32, (128, 128), 1)
        fold[...] = jnp.where(((li & 63) >> 1) == ((lj & 63) >> 1), 1.0, 0.0).astype(BF)
        wbT[pl.ds(1728, 64), :] = jnp.zeros((64, DP), BF)
        wobP[pl.ds(512, 64), :] = jnp.zeros((64, DP), BF)

    def xpose_w(w_ref, t_ref, c0, c1, kt):
        blk = w_ref[pl.ds(128 * kt, 128), pl.ds(c0, c1 - c0)]
        t_ref[kt, pl.ds(c0 // 2, (c1 - c0) // 2), :] = pltpu.bitcast(blk.T, U32)

    def gather_rows(t_ref, dst, src0, nh, dst0, kt):
        v = t_ref[kt, pl.ds(src0, nh, stride=9), :]
        dst.bitcast(U32)[pl.ds(dst0 // 2, nh), pl.ds(128 * kt, 128)] = v

    def prep_a(part, kt):
        for g in range(4):
            for c in range(9):
                gather_rows(ta, waT, part * 288 + 72 * g + c, 8, part * D + 144 * g + 16 * c, kt)

    def prep_b_x(kt, u):
        c0, c1 = ((0, 640), (640, 1152), (1152, 3 * D))[u]
        xpose_w(wb, tb, c0, c1, kt)

    def prep_b_g(kt, part):
        for c in range(8):
            gather_rows(tb, wbT, part * 288 + c, 32, part * 512 + 64 * c, kt)
        gather_rows(tb, wbT, part * 288 + 8, 32, (1536, 1664, 1600)[part], kt)

    def prep_wob_a(jt):
        w = min(128, D - 128 * jt)
        t2[jt, :, pl.ds(0, w)] = pltpu.bitcast(wob[:, pl.ds(128 * jt, w)], U32)

    def prep_wob_b(c):
        lane = jax.lax.broadcasted_iota(jnp.int32, (32, 128), 1)
        prev = None
        dst0 = 64 * c if c < 8 else 576
        for jt in range(5):
            v = t2[jt, pl.ds(c, 32, stride=9), :]
            if jt == 4:
                v = jnp.where(lane < 64, v, jnp.uint32(0))
            r = pltpu.roll(v, 64, 1)
            lo = jnp.zeros_like(r) if prev is None else prev
            wobP.bitcast(U32)[pl.ds(dst0 // 2, 32), pl.ds(128 * jt, 128)] = jnp.where(lane < 64, lo, r)
            prev = r

    def prep_woT(t):
        w = min(128, D - 128 * t)
        woT[:, pl.ds(128 * t, w)] = woa[pl.ds(128 * t, w), :].T

    def a_k(i, g):
        p0, n = P1[i]
        xs = xa[:, pl.ds(p0, n)]
        kT = jnp.dot(waT[pl.ds(D + 144 * g, 144), :], xs, preferred_element_type=F32)
        pks[i % 2][pl.ds(144 * g, 144), pl.ds(0, n)] = _phi(kT).astype(BF)

    def a_g(i, j):
        p0, n = P1[i]
        xs = xa[pl.ds(128 * j, 128), pl.ds(p0, n)]
        gp = jax.lax.dot_general(pks[i % 2][:, pl.ds(0, n)], xs, NT, preferred_element_type=F32)
        if i == 0:
            g_acc[:, pl.ds(128 * j, 128)] = gp
        else:
            g_acc[:, pl.ds(128 * j, 128)] += gp

    groups = [(0,), (0, 1), (1, 2), (2, 3), (3,)]
    krange = [(0, 256), (0, 384), (128, 512), (256, 576), (384, 576)]

    def a_z():
        zb[...] = jnp.broadcast_to(g_acc[:, pl.ds(D, 1)], (D, 128))

    def a_kv(j):
        w = min(128, D - 128 * j)
        wv = wa[:, pl.ds(2 * D + 128 * j, w)]
        for g in groups[j]:
            gb = g_acc[pl.ds(144 * g, 144), :].astype(BF)
            kv = jnp.dot(gb, wv, preferred_element_type=F32)
            r = jax.lax.broadcasted_iota(jnp.int32, (144, w), 0)
            n = jax.lax.broadcasted_iota(jnp.int32, (144, w), 1) + 128 * j
            lo = ((r & 15) >> 1) * DH + 144 * g
            kvm[pl.ds(144 * g, 144), pl.ds(128 * j, w)] = jnp.where((n >= lo) & (n < lo + DH), kv, 0.0).astype(BF)

    def a_m(j):
        w = min(128, D - 128 * j)
        k0, k1 = krange[j]
        m = jax.lax.dot_general(woT[:, pl.ds(k0, k1 - k0)], kvm[pl.ds(128 * j, w), pl.ds(k0, k1 - k0)], NT,
                                preferred_element_type=F32)
        mT[:, pl.ds(128 * j, w)] = m.astype(BF)

    cscale = (DH ** -0.5) * LOG2E
    NEG = -1e9 / (DH ** -0.5)

    def b_first_halo():
        for j in range(5):
            vb0[j, pl.ds(0, HALO), :] = jnp.broadcast_to(vb0[j, pl.ds(HALO, 1), :], (HALO, 128))

    def b_xn(i):
        vals["xn", i] = xb[:, pl.ds(i * RB, RB)].T

    def b_proj(i, p):
        c0, n = PP[p]
        rows = pl.ds(HALO, RB)
        res = jax.lax.dot_general(vals["xn", i], wbT[pl.ds(c0, n), :], NT, preferred_element_type=F32)
        for u in range(n // 128):
            v, t = res[:, 128 * u:128 * u + 128], c0 // 128 + u
            if t < 4:
                qbufs[i % 2][t] = v
            elif t < 8:
                kbufs[i % 2][t - 4, rows, :] = v
            elif t < 12:
                vbufs[i % 2][t - 8, rows, :] = v
            elif t == 12:
                vbufs[i % 2][4, rows, :] = v
            else:
                kbufs[i % 2][4, rows, :] = v

    def b_halo(i):
        if i == 0:
            return
        kbuf, vbuf = kbufs[i % 2], vbufs[i % 2]
        kp, vp = kbufs[(i - 1) % 2], vbufs[(i - 1) % 2]
        for j in range(5):
            kbuf[j, pl.ds(0, HALO), :] = kp[j, pl.ds(RB, HALO), :]
            vbuf[j, pl.ds(0, HALO), :] = vp[j, pl.ds(RB, HALO), :]

    def b_qk(i, c):
        kbuf, vbuf, qbuf = kbufs[i % 2], vbufs[i % 2], qbufs[i % 2]
        for r in range(c * FC, (c + 1) * FC, GR):
            q = [qbuf[j, pl.ds(r, GR), :] for j in range(4)] + [vbuf[4, pl.ds(HALO + r, GR), :]]
            accs = []
            for w in range(NW):
                rs = pl.ds(HALO + r - DIL * w, GR)
                a = q[0] * kbuf[0, rs, :]
                for j in range(1, 5):
                    a = a + q[j] * kbuf[j, rs, :]
                accs.append(a)
            accb[pl.ds(r * NW, GR * NW), :] = jnp.concatenate(accs, axis=0).astype(BF)

    def b_fold(i, c):
        for r in range(c * FC, (c + 1) * FC, FG):
            L = jnp.dot(accb[pl.ds(r * NW, FG * NW), :], fold[...], preferred_element_type=F32)
            for u in range(0, FG, GR):
                vals["L", i, r + u] = L[u * NW:(u + GR) * NW]

    def b_av(i, c):
        vbuf = vbufs[i % 2]
        for r in range(c * FC, (c + 1) * FC, GR):
            L = vals.pop(("L", i, r))
            ls = [L[w * GR:(w + 1) * GR] for w in range(NW)]
            if i == 0 and r == 0:
                row = jax.lax.broadcasted_iota(jnp.int32, (GR, 128), 0)
                ls = [ls[0]] + [jnp.where(row >= DIL * w, ls[w], NEG) for w in range(1, NW)]
            m01 = jnp.maximum(jnp.maximum(ls[0], ls[1]), jnp.maximum(ls[2], ls[3]))
            m23 = jnp.maximum(jnp.maximum(ls[4], ls[5]), jnp.maximum(ls[6], ls[7]))
            m = jnp.maximum(m01, m23)
            es = [jnp.exp2((l - m) * cscale) for l in ls]
            s = ((es[0] + es[1]) + (es[2] + es[3])) + ((es[4] + es[5]) + (es[6] + es[7]))
            rinv = pl.reciprocal(s, approx=True)
            os_ = []
            for j in range(5):
                o = es[0] * vbuf[j, pl.ds(HALO + r, GR), :]
                for w in range(1, NW):
                    o = o + es[w] * vbuf[j, pl.ds(HALO + r - DIL * w, GR), :]
                os_.append(o * rinv)
            obufs[i % 2][pl.ds(r, GR), :] = jnp.concatenate(os_, axis=1).astype(BF)

    def b_out(i, p):
        c0, n = BP[p]
        ob = jnp.dot(obufs[i % 2][...], wobP[:, pl.ds(c0, n)], preferred_element_type=F32)
        ob = ob.astype(BF)
        rows = pl.ds(i * RB, RB)
        if c0 == 0:
            outs[rows, pl.ds(D, n - 64)] = ob[:, 64:]
        else:
            outs[rows, pl.ds(512 + c0, n)] = ob

    def a_q(i, p):
        c0, n = AQP[p]
        xs = xa[:, pl.ds(i * RB, RB)]
        qT = jnp.dot(waT[pl.ds(c0, n), :], xs, preferred_element_type=F32)
        for u in range(0, n, 144):
            vals["q", i, (c0 + u) // 144] = qT[u:u + 144]

    def a_p(i, g, lt):
        pq = _phi(vals["q", i, g][:, 128 * lt:128 * lt + 128])
        par = jax.lax.broadcasted_iota(jnp.int32, (8, 128), 0) & 1
        halves = []
        for hf in range(2):
            t = None
            for c in range(9):
                r = 16 * c + 8 * hf
                u = pq[r:r + 8] * zb[pl.ds(144 * g + r, 8), :]
                t = u if t is None else t + u
            sw = jnp.where(par == 0, pltpu.roll(t, 7, 0), pltpu.roll(t, 1, 0))
            halves.append(pl.reciprocal(t + sw + 1e-6, approx=True))
        rinv = jnp.concatenate(halves, axis=0)
        pT = jnp.concatenate([pq[16 * c:16 * c + 16] * rinv for c in range(9)], axis=0)
        pbuf[pl.ds(144 * g, 144), pl.ds(128 * lt, 128)] = pT.astype(BF)

    def a_out(i, t):
        c0, n = AOP[t]
        vals["o", i, t] = jnp.dot(mT[pl.ds(c0, n), pl.ds(0, D)], pbuf[...],
                                  preferred_element_type=F32).astype(BF)

    def a_store(i, t):
        c0, n = AOP[t]
        o = vals.pop(("o", i, t))
        outs[pl.ds(i * RB, RB), pl.ds(c0, n)] = o.T

    for kt in range(5):
        c_wak[kt].wait()
        xpose_w(wa, ta, 512, 1152, kt)
        prep_a(1, kt)
    c_xa0.wait()
    for g in range(4):
        a_k(0, g)

    def wait1():
        c_xa2.wait()
        c_waq.wait()

    def wait3():
        for c in (c_wb, c_wob, c_woa, c_wav):
            c.wait()

    side = {k: [] for k in range(N1)}
    side[0] += [init_late]
    side[1] += [lambda kt=kt: (xpose_w(wa, ta, 0, 512, kt), prep_a(0, kt)) for kt in range(5)]
    wbt = []
    for kt in range(5):
        wbt += [lambda kt=kt, u=u: prep_b_x(kt, u) for u in range(3)]
        if kt >= 1:
            wbt += [lambda kt=kt, u=u: prep_b_g(kt - 1, u) for u in range(3)]
    wbt += [lambda u=u: prep_b_g(4, u) for u in range(3)]
    n3 = 24
    side[3] += wbt[:n3]
    late = [lambda jt=jt: prep_wob_a(jt) for jt in range(5)]
    late += [lambda c=c: prep_wob_b(c) for c in range(9)]
    late += [lambda t=t: prep_woT(t) for t in range(5)]
    rest = wbt[n3:]
    side[4] += [f for _, f in sorted([((k + .5) / len(rest), f) for k, f in enumerate(rest)] +
                                     [((k + .5) / len(late), f) for k, f in enumerate(late)], key=lambda t: t[0])]
    pre = {0: c_xa1.wait, 1: wait1, 2: c_xa3.wait, 3: wait3, 4: c_xb.wait}

    for i in range(N1):
        if i in pre:
            pre[i]()
        todo = side[i]
        n = len(todo)
        for j in range(5):
            if i + 1 < N1 and j < 4:
                a_k(i + 1, j)
            a_g(i, j)
            for f in todo[(j * n) // 5:((j + 1) * n) // 5]:
                f()

    b_xn(0)
    a_z()
    for p in range(len(PP)):
        b_proj(0, p)
        if p == 0:
            b_xn(1)

    b_first_halo()

    def T(i, name, *args):
        if 0 <= i < NB:
            fns[name](i, *args)

    def o_a(i):
        out_copy(i, 0, DP)

    def o_b(i):
        out_copy(i, DP, 2 * D - DP)

    fns = dict(P=b_proj, QK=b_qk, F=b_fold, AV=b_av, AQ=a_q, AP=a_p, BO=b_out, AO=a_out, AS=a_store,
               XN=b_xn, HL=b_halo, OA=o_a, OB=o_b, OC=lambda i, c0, n: out_copy(i, 128 * c0, 128 * n),
               KV=lambda i, j: a_kv(j) if i == 0 else None,
               MT=lambda i, j: a_m(j) if i == 0 else None)
    for i in range(NB + 1):
        for name, off, *args in make_plan({NB - 1: "PLAN_PRE", NB: "PLAN_LAST", 0: "PLAN_FIRST"}.get(i)):
            T(i + off, name, *args)
    for c in outc:
        c.wait()


_PLANS = {
    'PLAN': """
AQ:-1:0 KV:0:0 APG:-1:0 KV:0:1 AQ:-1:2 AQ:-1:3 AQ:-1:1 APG:-1:1
APG:-1:2 HL:0 QK:0:0 F:0:0 P:1:0 BO:-1:0 QK:0:1 APG:-1:3
F:0:1 BO:-1:1 AV:0:0 QK:0:2 F:0:2 BO:-1:2 OB:-1 AV:0:1
KV:0:2 QK:0:3 F:0:3 P:1:1 AV:0:3 AV:0:2 KV:0:3 QK:0:4
F:0:4 P:1:2 KV:0:4 QK:0:7 QK:0:5 P:1:4 F:0:5 P:1:3
P:1:5 AV:0:4 MT:0:1 AV:0:5 F:0:7 MT:0:0 QK:0:6 MT:0:3
F:0:6 AV:0:6 MT:0:2 AO:-1:0 P:1:6 AV:0:7 AO:-1:1 MT:0:4
XN:2 AS:-1:0 AO:-1:2 AS:-1:1 AS:-1:2 OA:-1
""",
    'PLAN_LAST': """
AQ:-1:0 AQ:-1:1 APG:-1:0 AQ:-1:2 APG:-1:1 AQ:-1:3 APG:-1:2 BO:-1:2
OC:-1:8:1 APG:-1:3 AO:-1:0 AO:-1:1 AS:-1:0 OC:-1:0:2 AO:-1:2 AS:-1:1
OC:-1:2:2 AS:-1:2 BO:-1:0 OC:-1:4:2 BO:-1:1 OC:-1:6:2
""",
}


def make_plan(special=None):
    out = []
    for tok in _PLANS.get(special, _PLANS["PLAN"]).split():
        name, *args = tok.split(":")
        args = [int(a) for a in args]
        if name == "APG":
            out += [("AP", args[0], args[1], lt) for lt in range(2)]
        else:
            out.append((name, *args))
    return out


def build():
    hbm = pl.BlockSpec(memory_space=pltpu.HBM)
    vm = pltpu.VMEM
    scratch = [
        vm((DP, S), BF), vm((DP, S), BF),
        vm((DP, 3 * D), BF), vm((DP, 3 * D), BF),
        vm((D, D), BF), vm((D, D), BF),
        vm((5, 864, 128), U32), vm((5, 864, 128), U32), vm((5, 288, 128), U32),
        vm((2 * D, DP), BF), vm((1792, DP), BF), vm((D, D), BF), vm((DP, DP), BF),
        vm((D, DP), F32), vm((D, DP), BF), vm((D, DP), BF), vm((D, 128), F32),
        vm((5, HALO + RB, 128), F32), vm((5, HALO + RB, 128), F32),
        vm((5, HALO + RB, 128), F32), vm((5, HALO + RB, 128), F32),
        vm((4, RB, 128), F32), vm((4, RB, 128), F32), vm((RB, DP), BF), vm((RB, DP), BF),
        vm((NW * RB, 128), BF),
        vm((D, R1), BF), vm((D, R1), BF), vm((D, RB), BF),
        vm((S, 2 * D), BF), vm((128, 128), BF),
        pltpu.SemaphoreType.DMA((16,)), pltpu.SemaphoreType.DMA((5 * NB,)),
    ]
    return pl.pallas_call(
        _kernel,
        out_shape=jax.ShapeDtypeStruct((S, 2 * D), BF),
        in_specs=[hbm] * 6,
        out_specs=hbm,
        scratch_shapes=scratch,
        compiler_params=pltpu.CompilerParams(vmem_limit_bytes=100 << 20),
    )


@jax.jit
def pallas_concat_heads__linear_attn_block__sliding_local_dilated__prompt_kernel(A_x, A_wqkv, A_wo, B_x, B_wqkv, B_wo):
    out = build()(A_x.reshape(S, D).T, A_wqkv, A_wo, B_x.reshape(S, D).T, B_wqkv, B_wo)
    return out.reshape(1, S, 2 * D)
```
